```python
import os as _os
_os.environ.setdefault("JAX_PLATFORMS", "cpu")
import jax
import jax.numpy as jnp

def _softmax(x, axis=-1):
    return jax.nn.softmax(x, axis=axis)
def _gelu(x):
    return jax.nn.gelu(x, approximate=True)
def _silu(x):
    return jax.nn.silu(x)
def _sigmoid(x):
    return jax.nn.sigmoid(x)
def _layernorm(x, axis=-1, eps=1e-5):
    m = jnp.mean(x, axis=axis, keepdims=True)
    v = jnp.var(x, axis=axis, keepdims=True)
    return (x - m) / jnp.sqrt(v + eps)
def _scatter_add(tgt, idx, src, axis=0):
    return tgt.at[idx].add(src)
def _segment_sum(src, seg, n):
    return jax.ops.segment_sum(src, seg, n)
class _Rng:
    def __init__(self, key):
        self._k = key
    def _next(self):
        self._k, sub = jax.random.split(self._k)
        return sub
    def normal(self, shape):
        return jax.random.normal(self._next(), shape, dtype=jnp.bfloat16)
    def randint(self, lo, hi, shape):
        return jax.random.randint(self._next(), shape, lo, hi, dtype=jnp.int32)
    def uniform(self, shape, lo=0.0, hi=1.0):
        return jax.random.uniform(self._next(), shape, jnp.bfloat16, lo, hi)
    def permutation(self, n):
        return jax.random.permutation(self._next(), n)


kernel_name = 'concat_heads__gqa_block_cached__gqa_block_cached__near_ridge'

def setup_inputs():
    _rng = _Rng(jax.random.key(int.from_bytes(__import__("os").urandom(4), "little")))
    _w = (lambda a: (lambda t: t.astype(jnp.bfloat16) if jnp.issubdtype(t.dtype, jnp.floating) else t)(jnp.asarray(a)))
    def _A_setup():
        B, Sq, D = 32, 48, 512
        Hq, Hkv, Sk, Dh = 32, 32, 48, 128
        assert Hq % Hkv == 0, (Hq, Hkv)
        return {
            "x": _w((lambda *s: _rng.normal(s) * 0.8)(B, Sq, D)),
            "k_cache": _w((lambda *s: _rng.normal(s) * 0.8)(B, Hkv, Sk, Dh)),
            "v_cache": _w((lambda *s: _rng.normal(s) * 0.05)(B, Hkv, Sk, Dh)),
            "wq": _w((lambda *s: _rng.normal(s) * 0.8)(D, Hq * Dh) * (D ** -0.5)),
            "wo": _w((lambda *s: _rng.normal(s) * 0.05)(Hq * Dh, D) * ((Hq * Dh) ** -0.5)),
        }
    _A_in = _A_setup()

    def _B_setup():
        B, Sq, D = 32, 48, 512
        Hq, Hkv, Sk, Dh = 32, 32, 48, 128
        assert Hq % Hkv == 0, (Hq, Hkv)
        return {
            "x": _w((lambda *s: _rng.normal(s) * 0.8)(B, Sq, D)),
            "k_cache": _w((lambda *s: _rng.normal(s) * 0.8)(B, Hkv, Sk, Dh)),
            "v_cache": _w((lambda *s: _rng.normal(s) * 0.05)(B, Hkv, Sk, Dh)),
            "wq": _w((lambda *s: _rng.normal(s) * 0.8)(D, Hq * Dh) * (D ** -0.5)),
            "wo": _w((lambda *s: _rng.normal(s) * 0.05)(Hq * Dh, D) * ((Hq * Dh) ** -0.5)),
        }
    _B_in = _B_setup()

    return {
        "A_x": _A_in["x"],
        "A_k_cache": _A_in["k_cache"],
        "A_v_cache": _A_in["v_cache"],
        "A_wq": _A_in["wq"],
        "A_wo": _A_in["wo"],
        "B_x": _B_in["x"],
        "B_k_cache": _B_in["k_cache"],
        "B_v_cache": _B_in["v_cache"],
        "B_wq": _B_in["wq"],
        "B_wo": _B_in["wo"],
    }

def reference(A_x, A_k_cache, A_v_cache, A_wq, A_wo, B_x, B_k_cache, B_v_cache, B_wq, B_wo):
    def _A_ref(x, k_cache, v_cache, wq, wo):
        B, Sq, D = x.shape
        Hq, Dh = 32, 128
        Hkv = k_cache.shape[1]
        rep = Hq // Hkv
        q = (lambda x, *d: x.transpose(*d))((x @ wq).reshape(B, Sq, Hq, Dh), 0, 2, 1, 3)
        k = jnp.repeat(k_cache, rep, axis=1)
        v = jnp.repeat(v_cache, rep, axis=1)
        scores = jnp.einsum("bhqd,bhkd->bhqk", q, k) * (Dh ** -0.5)
        p = _softmax(scores, axis=-1)
        o = jnp.einsum("bhqk,bhkd->bhqd", p, v)
        return (lambda x, *d: x.transpose(*d))(o, 0, 2, 1, 3).reshape(B, Sq, Hq * Dh) @ wo

    def _B_ref(x, k_cache, v_cache, wq, wo):
        B, Sq, D = x.shape
        Hq, Dh = 32, 128
        Hkv = k_cache.shape[1]
        rep = Hq // Hkv
        q = (lambda x, *d: x.transpose(*d))((x @ wq).reshape(B, Sq, Hq, Dh), 0, 2, 1, 3)
        k = jnp.repeat(k_cache, rep, axis=1)
        v = jnp.repeat(v_cache, rep, axis=1)
        scores = jnp.einsum("bhqd,bhkd->bhqk", q, k) * (Dh ** -0.5)
        p = _softmax(scores, axis=-1)
        o = jnp.einsum("bhqk,bhkd->bhqd", p, v)
        return (lambda x, *d: x.transpose(*d))(o, 0, 2, 1, 3).reshape(B, Sq, Hq * Dh) @ wo

    a = _A_ref(A_x, A_k_cache, A_v_cache, A_wq, A_wo)
    b = _B_ref(B_x, B_k_cache, B_v_cache, B_wq, B_wo)
    return jnp.concatenate([a, b], axis=-1)
```

```python
import os
import jax
import jax.numpy as jnp
from jax import lax
import jax.experimental.pallas as pl
import jax.experimental.pallas.tpu as pltpu

B, SQ, D = 32, 48, 512
H, SK, DH = 32, 48, 128
HG = 4
R = 4
PROF = int(os.environ.get('PROF', 0))
NS = H // HG
NT = 2 * NS
NC = B // R
NU = 2 * NC
CR = R * SQ
HR = CR // 2
SH = SQ // 2
M = B * SQ
W = HG * DH
KH = 256
RB = KH // NU
NBUF = 3
T_XB = 4
C = (DH ** -0.5) * 1.4426950408889634
f32 = jnp.float32
bf16 = jnp.bfloat16
u32 = jnp.uint32

S_X = 4 * NBUF
S_XB = S_X + 3
S_OA = S_XB + 1
S_OB = S_OA + 1
NSEM = S_OB + NC


class _Null:
    def __enter__(self): return self
    def __exit__(self, *a): return False


def scope(name):
    return jax.named_scope(name) if PROF else _Null()


def _recip(l):
    r = pl.reciprocal(l, approx=True)
    return r * (2.0 - l * r)


def pk(v):
    return pltpu.bitcast(v.astype(bf16), u32)


def up(v):
    return pltpu.bitcast(v, bf16)


def dot(a, b):
    return jnp.dot(a, b, preferred_element_type=f32)


def lhs_ops(a11, a12, a21, a22):
    return (a11 + a22, a21 + a22, a11, a22, a11 + a12, a21 - a11, a12 - a22)


def rhs_ops(b11, b12, b21, b22):
    return (b11 + b22, b11, b12 - b22, b21 - b11, b22, b11 + b12, b21 + b22)


def kernel(ax, ak, av, awq, awo, bx, bk, bv, bwq, bwo, out_hbm,
           x_buf, k_buf, v_buf, wq_buf, wo_buf, q_scr, q_alt, o_scr, xs, wqs, wos, acc, ostage, zero, sem):
    srcs = ((ax, ak, av, awq, awo), (bx, bk, bv, bwq, bwo))

    def _c0(hg):
        return hg * W if isinstance(hg, int) else pl.multiple_of(hg * W, W)

    def cp_wq(br, hg, slot):
        return pltpu.make_async_copy(srcs[br][3].at[:, pl.ds(_c0(hg), W)], wq_buf.at[slot], sem.at[4 * slot])

    def cp_k(br, hg, slot):
        return pltpu.make_async_copy(srcs[br][1].at[:, pl.ds(hg * HG, HG)], k_buf.at[slot], sem.at[4 * slot + 1])

    def cp_v(br, hg, slot):
        return pltpu.make_async_copy(srcs[br][2].at[:, pl.ds(hg * HG, HG)], v_buf.at[slot], sem.at[4 * slot + 2])

    def cp_wo(br, hg, slot):
        return pltpu.make_async_copy(srcs[br][4].at[pl.ds(_c0(hg), W), :], wo_buf.at[slot], sem.at[4 * slot + 3])

    XP = ((0, NC // 4), (NC // 4, NC // 2), (NC // 2, NC))

    def cp_xa(i):
        lo, hi = XP[i]
        sl = pl.ds(lo * CR, (hi - lo) * CR)
        return pltpu.make_async_copy(ax.at[sl], x_buf.at[0, sl], sem.at[S_X + i])

    def cp_xb():
        return pltpu.make_async_copy(bx, x_buf.at[1], sem.at[S_XB])

    def cp_oa():
        return pltpu.make_async_copy(ostage.at[0], out_hbm.at[:, pl.ds(0, D)], sem.at[S_OA])

    def cp_ob(c):
        sl = pl.ds(c * CR, CR)
        return pltpu.make_async_copy(ostage.at[1, sl], out_hbm.at[sl, pl.ds(D, D)], sem.at[S_OB + c])

    def issue_packet_static(p):
        slot = p % NBUF
        cp_wq(0, p + 2, slot).start()
        cp_k(0, p, slot).start()
        cp_v(0, p, slot).start()
        cp_wo(0, p, slot).start()

    def wait_packet(slot):
        cp_wq(0, 0, slot).wait()
        cp_k(0, 0, slot).wait()
        cp_v(0, 0, slot).wait()
        cp_wo(0, 0, slot).wait()

    def issue_packet_dyn(p):
        slot = p % NBUF

        @pl.when(p + 2 < NS)
        def _():
            cp_wq(0, p + 2, slot).start()

        @pl.when(jnp.logical_and(p + 2 >= NS, p + 2 < NT))
        def _():
            cp_wq(1, p + 2 - NS, slot).start()

        @pl.when(p + 2 == NT)
        def _():
            for j, h in enumerate((0, 2, 1, 3)):
                pltpu.make_async_copy(bwo.at[pl.ds((NS - 1) * W + h * DH, DH), :],
                                      wq_buf.at[slot, pl.ds(j * DH, DH), :], sem.at[4 * slot]).start()

        @pl.when(p < NS)
        def _():
            cp_k(0, p, slot).start()
            cp_v(0, p, slot).start()
            cp_wo(0, p, slot).start()

        @pl.when(jnp.logical_and(p >= NS, p < NT))
        def _():
            cp_k(1, p - NS, slot).start()
            cp_v(1, p - NS, slot).start()

        @pl.when(jnp.logical_and(p >= NS, p < NT - 1))
        def _():
            cp_wo(1, p - NS, slot).start()

    last = {}

    def anchor():
        z = pltpu.bitcast(pltpu.bitcast(last['v'][:8, :DH], u32) & zero[...], f32)
        z = jnp.concatenate([z, z], axis=1)
        return jnp.concatenate([z, z], axis=0)

    def w_sums(w_buf, slot, dst, j, perm):
        r = j * RB
        r0, r1 = ((r // DH) * 2 * DH + r % DH, (r // DH) * 2 * DH + r % DH + DH) if perm else (r, KH + r)
        t = w_buf[slot, r0:r0 + RB, :].astype(f32)
        bt = w_buf[slot, r1:r1 + RB, :].astype(f32)
        ev = lambda v: jnp.concatenate([v[:, :DH], v[:, 2 * DH:3 * DH]], axis=1)
        od = lambda v: jnp.concatenate([v[:, DH:2 * DH], v[:, 3 * DH:]], axis=1)
        z = anchor()
        ops = rhs_ops(ev(t) + z, od(t), ev(bt), od(bt) + z)
        dst[r // 2:(r + RB) // 2, :] = pk(jnp.concatenate(ops, axis=1))

    def wq_sums(slot, dst, j):
        w_sums(wq_buf, slot, dst, j, False)

    def wo_sums(slot, dst, j):
        w_sums(wo_buf, slot, dst, j, True)

    def x_sums(br, c):
        dst = xs.at[br]
        for b in range(c * R, (c + 1) * R, 2):
            for kt in range(2):
                def blk(half, c0):
                    cols = slice(c0 + kt * DH, c0 + (kt + 1) * DH)
                    v = [x_buf[br, (b + j) * SQ:(b + j + 1) * SQ, cols].astype(f32) for j in range(2)]
                    return jnp.concatenate([v[0][half * SH:(half + 1) * SH], v[1][half * SH:(half + 1) * SH]], axis=0)
                ops = lhs_ops(blk(0, 0), blk(0, KH), blk(1, 0), blk(1, KH))
                dst[b * SH // 2:(b + 2) * SH // 2, kt * 7 * DH:(kt + 1) * 7 * DH] = pk(jnp.concatenate(ops, axis=1))

    def lhs_load(ref, c, i):
        rows = slice(c * HR // 2, (c + 1) * HR // 2)
        return up(jnp.concatenate([ref[rows, (kt * 7 + i) * DH:(kt * 7 + i + 1) * DH] for kt in range(2)], axis=1))

    def rhs_load(ref, nt, i):
        return up(ref[:, i * KH + nt * DH:i * KH + (nt + 1) * DH])

    def strassen(lhs, rhs, finish):
        st = {}

        def p1():
            m2 = dot(lhs(1), rhs(1))
            m4 = dot(lhs(3), rhs(3))
            m3 = dot(lhs(2), rhs(2))
            m5 = dot(lhs(4), rhs(4))
            st['c21'] = m2 + m4
            st['c12'] = m3 + m5
            st['t11'] = m4 - m5
            st['t22'] = m3 - m2
            last['a'] = m2

        def p2():
            m1 = dot(lhs(0), rhs(0))
            m7 = dot(lhs(6), rhs(6))
            m6 = dot(lhs(5), rhs(5))
            finish(st['t11'] + (m1 + m7), st['c12'], st['c21'], st['t22'] + (m1 + m6))
        return p1, p2

    def interleave(top, bot):
        pieces = []
        for r in range(R):
            pieces += [top[r * SH:(r + 1) * SH], bot[r * SH:(r + 1) * SH]]
        return jnp.concatenate(pieces, axis=0)

    def A_plain(u, slot, q_dst):
        c, nt = divmod(u, 2)
        st = {}

        def p1():
            st['q'] = dot(x_buf[0, c * CR:(c + 1) * CR, :], wq_buf[slot, :, 2 * nt * DH:(2 * nt + 1) * DH])
            last['a'] = st['q']

        def p2():
            q1 = dot(x_buf[0, c * CR:(c + 1) * CR, :], wq_buf[slot, :, (2 * nt + 1) * DH:(2 * nt + 2) * DH])
            last['a'] = q1
            q_dst[c * HR:(c + 1) * HR, nt * KH:(nt + 1) * KH] = pk(jnp.concatenate([st['q'], q1], axis=1))
        return p1, p2

    def A_str(u, xbr, q_dst, wsrc):
        c, nt = divmod(u, 2)

        def finish(c11, c12, c21, c22):
            q = jnp.concatenate([interleave(c11, c21), interleave(c12, c22)], axis=1)
            q_dst[c * HR:(c + 1) * HR, nt * KH:(nt + 1) * KH] = pk(q)
        return strassen(lambda i: lhs_load(xs.at[xbr], c, i), lambda i: rhs_load(wsrc, nt, i), finish)

    def Bq(u, r2, slot, q_src, P):
        c, nt = divmod(u, 2)
        for r in range(2):
            b = c * R + 2 * r2 + r
            for h in (2 * nt, 2 * nt + 1):
                qq = up(q_src[b * SH:(b + 1) * SH, h * DH:(h + 1) * DH])
                s = lax.dot_general(qq, k_buf[slot, b, h], (((1,), (1,)), ((), ())), preferred_element_type=f32)
                m = jnp.max(s, axis=-1, keepdims=True)
                p = jnp.exp2((s - m) * C)
                l = jnp.sum(p, axis=-1, keepdims=True)
                P[(b, h)] = (p * _recip(l)).astype(bf16)

    def Cq(u, r2, slot, P):
        c, nt = divmod(u, 2)
        b0 = c * R + 2 * r2
        o = [[dot(P.pop((b0 + r, h)), v_buf[slot, b0 + r, h]) for h in (2 * nt, 2 * nt + 1)] for r in range(2)]
        last['c', r2] = o[0][0]
        cat = lambda j, half: jnp.concatenate(
            [o[0][j][half * SH:(half + 1) * SH], o[1][j][half * SH:(half + 1) * SH]], axis=0)
        ops = lhs_ops(cat(0, 0), cat(1, 0), cat(0, 1), cat(1, 1))
        o_scr[b0 * SH // 2:(b0 + 2) * SH // 2, nt * 7 * DH:(nt + 1) * 7 * DH] = pk(jnp.concatenate(ops, axis=1))

    def D_str(u, abr, wsrc, first=False, keep=True, stage=False, after=None):
        c, nt = divmod(u, 2)
        hs = slice(c * HR, (c + 1) * HR)
        cols = slice(nt * KH, (nt + 1) * KH)

        def finish(c11, c12, c21, c22):
            top = jnp.concatenate([c11, c12], axis=1)
            bot = jnp.concatenate([c21, c22], axis=1)
            if not first:
                top = acc[abr, 0, hs, cols] + top
                bot = acc[abr, 1, hs, cols] + bot
            if keep:
                acc[abr, 0, hs, cols] = top
                acc[abr, 1, hs, cols] = bot
            if stage:
                ostage[abr, c * CR:(c + 1) * CR, cols] = interleave(top, bot).astype(bf16)
            if after is not None:
                after()
        return strassen(lambda i: lhs_load(o_scr, c, i), lambda i: rhs_load(wsrc, nt, i), finish)

    def run2(parts):
        parts[0]()
        parts[1]()

    NOP = (lambda: None, lambda: None)

    def step(slot, q_src, lagC, fillB, fillC, tailfill, sums):
        P = {}
        for k in list(last):
            del last[k]
        for u in range(NU + lagC):
            fb = fillB(u) or NOP
            fc = fillC(u) or NOP
            if u < NU:
                Bq(u, 0, slot, q_src, P)
            fb[0]()
            if u < NU:
                Bq(u, 1, slot, q_src, P)
                fb[1]()
            if u >= lagC:
                Cq(u - lagC, 0, slot, P)
            fc[0]()
            if u >= lagC:
                Cq(u - lagC, 1, slot, P)
            fc[1]()
            if u >= NU:
                fb[1]()
            sums(u)
        for f in tailfill:
            run2(f)

    def rng(f, lo=0):
        return lambda u: f(u) if lo <= u < NU else None

    def step_sums(slot, wq_dst, wo_dst, lagC, extra=None):
        def sums(u):
            if extra is not None:
                extra(u)
            if u < lagC:
                return
            js = [u - lagC] if u - lagC < NU - 2 else []
            if u - lagC == NU - 4:
                js.append(NU - 2)
            if u - lagC == NU - 3:
                js.append(NU - 1)
            for j in js:
                if wq_dst is not None:
                    last['v'] = last['c', 0]
                    wq_sums(slot, wq_dst, j)
                if wo_dst is not None:
                    last['v'] = last['c', 1]
                    wo_sums(slot, wo_dst, j)
        return sums

    cp_wq(0, 0, 2).start()
    cp_xa(0).start()
    cp_xa(1).start()
    cp_wq(0, 1, 1).start()
    cp_xa(2).start()
    issue_packet_static(0)
    acc[1] = jnp.zeros((2, M // 2, D), f32)
    zero[...] = jnp.zeros((8, DH), u32)

    def plain_with_sums(units, slot, q_dst, w_dst):
        per = NU // (2 * len(units))
        j = 0
        for u in units:
            for part in A_plain(u, slot, q_dst):
                part()
                last['v'] = last['a']
                for _ in range(per):
                    wq_sums(slot, w_dst, j)
                    j += 1

    with scope('w1'):
        cp_wq(0, 0, 2).wait()
        cp_xa(0).wait()
    with scope('s1'):
        plain_with_sums(range(0, 4), 2, q_scr, wqs.at[0])
    with scope('w2'):
        cp_xa(1).wait()
        cp_wq(0, 1, 1).wait()
    with scope('s2'):
        plain_with_sums(range(0, 4), 1, q_alt, wos.at[0])
        for u in range(4, 8):
            if u % 2 == 0:
                x_sums(0, u // 2)
            run2(A_str(u, 0, q_scr, wqs.at[0]))
    with scope('w3'):
        cp_xa(2).wait()
        cp_wq(0, 0, 0).wait()
    with scope('s3'):
        issue_packet_static(1)
        issue_packet_static(2)
        cp_xb().start()
        j = 0
        work = [(u, q_alt, wos.at[0]) for u in range(4, 8)]
        for c in range(4, NC):
            work += [(2 * c, q_scr, wqs.at[0]), (2 * c + 1, q_scr, wqs.at[0]),
                     (2 * c, q_alt, wos.at[0]), (2 * c + 1, q_alt, wos.at[0])]
        for n, (u, qd, ws) in enumerate(work):
            if n >= 4 and n % 4 == 0:
                x_sums(0, u // 2)
            run2(A_str(u, 0, qd, ws))
            if j < NU:
                last['v'] = last['a']
                wq_sums(0, wqs.at[1], j)
                j += 1
    with scope('w4'):
        cp_k(0, 0, 0).wait()
        cp_v(0, 0, 0).wait()
        cp_wo(0, 0, 0).wait()
    with scope('s4'):
        x_sums(0, 0)
        x_sums(0, 1)
        step(0, q_scr, 1, lambda u: A_str(u - 1, 0, q_scr, wqs.at[1]) if u >= 1 else None,
             lambda u: None, [], step_sums(0, None, wos.at[1], 1))
    with scope('w5'):
        wait_packet(1)
    with scope('s5'):
        issue_packet_static(3)
        dd = lambda u: D_str(u, 0, wos.at[1], first=True)
        step(1, q_alt, 2, lambda u: dd(u) if u < 2 else None, rng(dd, 2), [],
             step_sums(1, wqs.at[2], wos.at[2], 2))

    def body(t, carry):
        slot = t % NBUF

        @pl.when(t == T_XB)
        def _():
            cp_xb().wait()
            for c in range(NC):
                x_sums(1, c)

        wait_packet(slot)
        xbr = (t + 1) // NS
        abr = (t - 1) // NS
        wqw = wqs.at[pl.ds(t, 2)]
        wow = wos.at[pl.ds(t, 2)]

        def extra(u):
            if u == 1:
                issue_packet_dyn(t + 2)

                @pl.when(t == NS + 1)
                def _():
                    cp_oa().start()

        dd = lambda u: D_str(u, abr, wow.at[0], stage=True)
        with scope('body'):
            step(slot, q_scr, 1,
                 lambda u: A_str(u - 1, xbr, q_scr, wqw.at[0]) if u >= 1 else dd(0),
                 lambda u: dd(u + 1) if u + 1 < NU else None, [],
                 step_sums(slot, wqw.at[1], wow.at[1], 1, extra))
        return carry

    lax.fori_loop(2, NT - 1, body, 0)

    t = NT - 1
    slot = t % NBUF
    with scope('w6'):
        cp_k(0, 0, slot).wait()
        cp_v(0, 0, slot).wait()
    with scope('tail'):
        d14 = lambda u: D_str(u, 1, wos.at[t])
        d15 = lambda u: D_str(u, 1, wqs.at[t], keep=False, stage=True,
                              after=((lambda: cp_ob(u // 2).start()) if u % 2 else None))
        step(slot, q_scr, 2, rng(d14), lambda u: d15(u - 5) if u >= 5 else None,
             [d15(u) for u in range(NU - 3, NU)], lambda u: None)
    with scope('wout'):
        cp_oa().wait()
        for c in range(NC):
            cp_ob(c).wait()


@jax.jit
def pallas_concat_heads__gqa_block_cached__gqa_block_cached__near_ridge_kernel(
    A_x, A_k_cache, A_v_cache, A_wq, A_wo, B_x, B_k_cache, B_v_cache, B_wq, B_wo):
    out = pl.pallas_call(
        kernel,
        in_specs=[pl.BlockSpec(memory_space=pl.ANY)] * 10,
        out_specs=pl.BlockSpec(memory_space=pl.ANY),
        out_shape=jax.ShapeDtypeStruct((M, 2 * D), bf16),
        scratch_shapes=[
            pltpu.VMEM((2, M, D), bf16),
            pltpu.VMEM((NBUF, B, HG, SK, DH), bf16),
            pltpu.VMEM((NBUF, B, HG, SK, DH), bf16),
            pltpu.VMEM((NBUF, D, W), bf16),
            pltpu.VMEM((NBUF, W, D), bf16),
            pltpu.VMEM((M // 2, W), u32),
            pltpu.VMEM((M // 2, W), u32),
            pltpu.VMEM((M // 4, 7 * KH), u32),
            pltpu.VMEM((2, M // 4, 7 * KH), u32),
            pltpu.VMEM((NT, KH // 2, 7 * KH), u32),
            pltpu.VMEM((NT, KH // 2, 7 * KH), u32),
            pltpu.VMEM((2, 2, M // 2, D), f32),
            pltpu.VMEM((2, M, D), bf16),
            pltpu.VMEM((8, DH), u32),
            pltpu.SemaphoreType.DMA((NSEM,)),
        ],
        compiler_params=pltpu.CompilerParams(
            vmem_limit_bytes=100 * 1024 * 1024,
            disable_bounds_checks=True, disable_semaphore_checks=True),
    )(A_x.reshape(M, D), A_k_cache, A_v_cache, A_wq, A_wo,
      B_x.reshape(M, D), B_k_cache, B_v_cache, B_wq, B_wo)
    return out.reshape(B, SQ, 2 * D)
```

```python
import jax
import jax.numpy as jnp
from jax import lax
import jax.experimental.pallas as pl
import jax.experimental.pallas.tpu as pltpu

B, SQ, D = 32, 48, 512
H, SK, DH = 32, 48, 128
HG = 4
R = 4
NS = H // HG
NT = 2 * NS
NC = B // R
NU = 2 * NC
NSC = NC // 2
ND = 7 * NSC
CR = R * SQ
HR = CR // 2
SH = SQ // 2
M = B * SQ
MQ = M // 4
SR = MQ // NSC
W = HG * DH
KH = 256
RB = 16
NBUF = 4
T0 = 3
T_XB = 5
LOGIT_LIMIT = 5.0
SCALE = DH ** -0.5
EXP2_SCALE = SCALE * 1.4426950408889634
f32 = jnp.float32
bf16 = jnp.bfloat16
u32 = jnp.uint32

S_X = 4 * NBUF
S_XB = S_X + 4
S_O = S_XB + 1
NSEM = S_O + 4 * NSC + 3

LHS_TERMS = (((0, 0), (1, 1), 1), ((1, 0), (1, 1), 1), ((0, 0), None, 0), ((1, 1), None, 0),
             ((0, 0), (0, 1), 1), ((1, 0), (0, 0), -1), ((0, 1), (1, 1), -1))
RHS_TERMS = (((0, 0), (1, 1), 1), ((0, 0), None, 0), ((0, 1), (1, 1), -1), ((1, 0), (0, 0), -1),
             ((1, 1), None, 0), ((0, 0), (0, 1), 1), ((1, 0), (1, 1), 1))
IORD = (1, 3, 4, 6, 0, 2, 5)
GROUPS = ((0, 0), (0, 1), (0, 2), (1, 0), (1, 1), (1, 2))


def _pack(v):
    return pltpu.bitcast(v.astype(bf16), u32)


def _unpack(v):
    return pltpu.bitcast(v, bf16)


def _dot(a, b):
    return jnp.dot(a, b, preferred_element_type=f32)


def _lhs_ops(a11, a12, a21, a22):
    return (a11 + a22, a21 + a22, a11, a22, a11 + a12, a21 - a11, a12 - a22)


def _rhs_ops(b11, b12, b21, b22):
    return (b11 + b22, b11, b12 - b22, b21 - b11, b22, b11 + b12, b21 + b22)


def _outer_combine(mm, half, z=None):
    shared = mm(3 if half == 0 else 2)
    if z is not None:
        shared = shared + z
    if half == 0:
        top, bot = (mm(0) + shared) + (mm(6) - mm(4)), mm(1) + shared
    else:
        top, bot = shared + mm(4), (mm(0) - mm(1)) + (shared + mm(5))
    return jnp.concatenate([top, bot], axis=0)


def _softmax(qq, kk):
    s = lax.dot_general(qq, kk, (((1,), (1,)), ((), ())), preferred_element_type=f32)
    s = jnp.concatenate([s, jnp.full((SQ, DH - SK), -jnp.inf, f32)], axis=1)
    m = jnp.max(s, axis=-1, keepdims=True)
    p = jnp.exp2((s - m) * EXP2_SCALE)
    l = jnp.sum(p, axis=-1, keepdims=True)
    r = pl.reciprocal(l, approx=True)
    r = r * (2.0 - l * r)
    return p * r, m


def _aligned(v, n):
    return v if isinstance(v, int) else pl.multiple_of(v, n)


def _kernel(ax, ak, av, awq, awo, bx, bk, bv, bwq, bwo, out_hbm,
            x_buf, k_buf, v_buf, wq_buf, wo_buf, q_scr, q_alt, p_scr, o_scr, o_alt, xs, ws,
            qm, qm1, qm2, acc, ostage, gmax, zero, flag, sem):
    srcs = ((ax, ak, av, awq, awo), (bx, bk, bv, bwq, bwo))

    def cp_wq(br, hg, slot):
        return pltpu.make_async_copy(srcs[br][3].at[:, pl.ds(_aligned(hg * W, W), W)],
                                     wq_buf.at[slot], sem.at[4 * slot])

    def cp_k(br, hg, slot):
        return pltpu.make_async_copy(srcs[br][1].at[:, pl.ds(hg * HG, HG)],
                                     k_buf.at[slot], sem.at[4 * slot + 1])

    def cp_v(br, hg, slot):
        return pltpu.make_async_copy(srcs[br][2].at[:, pl.ds(hg * HG, HG)],
                                     v_buf.at[slot], sem.at[4 * slot + 2])

    def cp_wo(br, hg, slot):
        return pltpu.make_async_copy(srcs[br][4].at[pl.ds(_aligned(hg * W, W), W), :],
                                     wo_buf.at[slot], sem.at[4 * slot + 3])

    def cp_xa(i):
        sl = pl.ds(_aligned(i * 2 * CR, 2 * CR), 2 * CR)
        return pltpu.make_async_copy(ax.at[sl], x_buf.at[0, sl], sem.at[S_X + i])

    def cp_xb():
        return pltpu.make_async_copy(bx, x_buf.at[1], sem.at[S_XB])

    def cp_out(br, sc, half, pr=None):
        if pr is None:
            rows, si = pl.ds(sc * 2 * CR, 2 * CR), (br * NSC + sc) * 2 + half
        else:
            rows, si = pl.ds(sc * 2 * CR + pr * 2 * SQ, 2 * SQ), 4 * NSC - 1 + pr
        return pltpu.make_async_copy(ostage.at[br, rows, pl.ds(half * KH, KH)],
                                     out_hbm.at[rows, pl.ds(br * D + half * KH, KH)],
                                     sem.at[S_O + si])

    def is_last(br, sc, half):
        return (br, sc, half) == (1, NSC - 1, 1)

    def issue_packet_static(p):
        slot = p % NBUF
        cp_wq(0, p + 2, slot).start()
        cp_k(0, p, slot).start()
        cp_v(0, p - 1, slot).start()
        cp_wo(0, p - 1, slot).start()

    def wait_packet(slot):
        cp_wq(0, 0, slot).wait()
        cp_k(0, 0, slot).wait()
        cp_v(0, 0, slot).wait()
        cp_wo(0, 0, slot).wait()

    def issue_packet_dyn(p):
        slot = p & (NBUF - 1)

        @pl.when(p + 2 < NS)
        def _():
            cp_wq(0, p + 2, slot).start()

        @pl.when(jnp.logical_and(p + 2 >= NS, p + 2 < NT))
        def _():
            cp_wq(1, p + 2 - NS, slot).start()

        @pl.when(p + 2 == NT)
        def _():
            pltpu.make_async_copy(bwo.at[pl.ds((NS - 2) * W, W), :], wq_buf.at[slot],
                                  sem.at[4 * slot]).start()

        @pl.when(p < NS)
        def _():
            cp_k(0, p, slot).start()

        @pl.when(jnp.logical_and(p >= NS, p < NT))
        def _():
            cp_k(1, p - NS, slot).start()

        @pl.when(p - 1 < NS)
        def _():
            cp_v(0, p - 1, slot).start()
            cp_wo(0, p - 1, slot).start()

        @pl.when(p - 1 >= NS)
        def _():
            cp_v(1, p - 1 - NS, slot).start()

        @pl.when(jnp.logical_and(p - 1 >= NS, p != NT - 1))
        def _():
            cp_wo(1, p - 1 - NS, slot).start()

    last = {}

    def anchor(v, rows, cols, k=0):
        z = pltpu.bitcast(pltpu.bitcast(v[8 * k:8 * k + 8, :DH], u32) & zero[0], f32)
        z = jnp.concatenate([z] * (cols // DH), axis=1)
        return jnp.concatenate([z] * (rows // 8), axis=0)

    def meter(todo, count):
        src = last['f']
        n = src.shape[0] // 8
        for k in range(count):
            if todo:
                todo.pop(0)(anchor(src, RB, KH, ((k + 1) * n) // count - 1))

    def w_sums(w, dst, j, i, z):
        r = j * RB

        def quad(k1, n1):
            return [w[(2 * k1 + k2) * DH + r:(2 * k1 + k2) * DH + r + RB,
                      n1 * KH:(n1 + 1) * KH].astype(f32) for k2 in range(2)]
        ta, tb, sg = RHS_TERMS[i]
        v = [x + z for x in quad(*ta)]
        if tb is not None:
            v = [x + y if sg > 0 else x - y for x, y in zip(v, quad(*tb))]
        ops = _rhs_ops(v[0][:, :DH], v[0][:, DH:], v[1][:, :DH], v[1][:, DH:])
        dst[r // 2:(r + RB) // 2, i * 7 * DH:(i + 1) * 7 * DH] = _pack(jnp.concatenate(ops, axis=1))

    def w_todo(w, dst):
        return [(lambda z, j=j, i=i: w_sums(w, dst, j, i, z))
                for j in range(DH // RB) for i in range(7)]

    def lhs_group(blk, i, z, dst, r0, nrows):
        ta, tb, sg = LHS_TERMS[i]
        v = {}
        for m2 in range(2):
            for k2 in range(2):
                x = blk(*ta, m2, k2)
                if z is not None and m2 == k2:
                    x = x + z
                if tb is not None:
                    y = blk(*tb, m2, k2)
                    x = x + y if sg > 0 else x - y
                v[m2, k2] = x
        ops = _lhs_ops(v[0, 0], v[0, 1], v[1, 0], v[1, 1])
        dst[r0 // 2:(r0 + nrows) // 2, i * 7 * DH:(i + 1) * 7 * DH] = _pack(jnp.concatenate(ops, axis=1))

    def x_ops(br, c, tile, z=None, outer=range(7)):
        grp = GROUPS[2 * tile:2 * tile + 2]
        xc = x_buf.at[br, pl.ds(_aligned(c * CR, CR), CR)]
        xd = xs.at[br, pl.ds(_aligned(c * SH, SH), SH)]

        def blk(m1, k1, m2, k2):
            out = []
            for q, g in grp:
                r = (2 * q + m2) * SQ + m1 * SH + 8 * g
                out.append(xc[r:r + 8, k1 * KH:(k1 + 1) * KH].astype(f32)[:, k2 * DH:(k2 + 1) * DH])
            return jnp.concatenate(out, axis=0)
        for i in outer:
            lhs_group(blk, i, None if z is None else z[:, :DH], xd, 16 * tile, 16)

    def x_todo(c0):
        return [(lambda z, c=c, tile=tile, i=i: x_ops(0, c0 + c, tile, z, (i,)))
                for c in range(2) for tile in range(3) for i in range(7)]

    def a_plain(u, slot, q_dst, x_src):
        c, nt = divmod(u, 2)
        st = {}

        def p1():
            st['q'] = _dot(x_src[c * CR:(c + 1) * CR, :], wq_buf[slot, :, 2 * nt * DH:(2 * nt + 1) * DH])
            last['f'] = st['q']

        def p2():
            q1 = _dot(x_src[c * CR:(c + 1) * CR, :], wq_buf[slot, :, (2 * nt + 1) * DH:(2 * nt + 2) * DH])
            last['f'] = q1
            q_dst[c * HR:(c + 1) * HR, nt * KH:(nt + 1) * KH] = _pack(jnp.concatenate([st['q'], q1], axis=1))
        return p1, p2

    def stage_b(b, slot, q_src):
        q_src = q_src(b)
        if len(q_src.shape) == 4:
            hs = slice((b // 2) * SH, (b // 2 + 1) * SH)
            vals = [q_src[i, b % 2, hs, :] for i in range(7)]
            qh = [_outer_combine(lambda i: vals[i], half) for half in range(2)]
            qs = [qh[h // 2][:, (h % 2) * DH:(h % 2 + 1) * DH].astype(bf16) for h in range(HG)]
        else:
            qs = [_unpack(q_src[b * SH:(b + 1) * SH, h * DH:(h + 1) * DH]) for h in range(HG)]
        ps, g = [], None
        for h in range(HG):
            p, m = _softmax(qs[h], k_buf[slot, b, h])
            ps.append(p)
            am = jnp.abs(m)
            for r in range(0, SQ, 8):
                g = am[r:r + 8] if g is None else jnp.maximum(g, am[r:r + 8])
        p_scr[b * SH:(b + 1) * SH, :] = _pack(jnp.concatenate(ps, axis=1))
        gmax[b] = jnp.maximum(gmax[b], jnp.broadcast_to(g, (8, DH)))

    o_val = {}

    def stage_c(b, slot):
        for h in range(HG):
            p = _unpack(p_scr[b * SH:(b + 1) * SH, h * DH:(h + 1) * DH])[:, :SK]
            o_val[b, h] = _dot(p, v_buf[slot, b, h])

    def c_tile(c, tile, o_dst):
        anc = last['f']
        grp = GROUPS[2 * tile:2 * tile + 2]
        n = anc.shape[0] // 8

        def blk(m1, k1, m2, k2):
            return jnp.concatenate(
                [o_val[c * R + 2 * q + m2, 2 * k1 + k2][m1 * SH + 8 * g:m1 * SH + 8 * g + 8]
                 for q, g in grp], axis=0)
        for i in range(7):
            lhs_group(blk, i, anchor(anc, 16, DH, (i * n) // 7), o_dst, c * SQ + 16 * tile, 16)

    def piece(n, pairs, dst, accumulate, after=None):
        sc, i = n // 7, IORD[n % 7]
        rows = slice(sc * SR // 2, (sc + 1) * SR // 2)
        hs = slice(sc * SR, (sc + 1) * SR)

        def mm(k):
            cols = slice((i * 7 + k) * DH, (i * 7 + k + 1) * DH)
            return _dot(_unpack(jnp.concatenate([o[rows, cols] for o, _ in pairs], axis=1)),
                        _unpack(jnp.concatenate([w[:, cols] for _, w in pairs], axis=0)))

        def run():
            m2, m4, m3, m5 = mm(1), mm(3), mm(2), mm(4)
            t11, t22, s34 = m4 - m5, m3 - m2, m3 + m4
            c21, c12 = s34 - t22, s34 - t11
            m1, m7, m6 = mm(0), mm(6), mm(5)
            last['f'] = jnp.concatenate([m2, m1], axis=0)
            top = jnp.concatenate([t11 + (m1 + m7), c12], axis=1)
            bot = jnp.concatenate([c21, t22 + (m1 + m6)], axis=1)
            if accumulate:
                top, bot = dst[i, 0, hs, :] + top, dst[i, 1, hs, :] + bot
            dst[i, 0, hs, :] = top
            dst[i, 1, hs, :] = bot
            if after is not None:
                after()
        return run

    def combine(br, sc, half, pin=False):
        anc = last['f']
        for pr in range(4):
            hs = slice(sc * SR + pr * SH, sc * SR + (pr + 1) * SH)
            for m2 in range(2):
                z = anchor(anc, SH, KH, 3 * (2 * pr + m2)) if pin else None
                v = _outer_combine(lambda i: acc[br, i, m2, hs, :], half, z)
                b = sc * 8 + 2 * pr + m2
                ostage[br, b * SQ:(b + 1) * SQ, half * KH:(half + 1) * KH] = v.astype(bf16)
            if is_last(br, sc, half):
                cp_out(br, sc, half, pr).start()
        if not is_last(br, sc, half):
            cp_out(br, sc, half).start()

    def run_slots(ops, fills):
        for u in range(len(fills)):
            for op, fl in zip(ops(u), fills[u]):
                if op is not None:
                    op()
                for f in fl:
                    f()

    def empty_fills():
        return [[[], [], [], []] for _ in range(NU + 1)]

    def cb_ops(slot, q_src):
        def ops(u):
            if u >= NU:
                return [None] * 4
            out = [lambda: stage_c(2 * u, slot), lambda: stage_c(2 * u + 1, slot)]
            if q_src is None:
                return out + [None, None]
            return out + [lambda: stage_b(2 * u, slot, q_src), lambda: stage_b(2 * u + 1, slot, q_src)]
        return ops

    def tile_fills(fills, o_dst):
        for u in range(NU):
            if u % 2 == 0:
                fills[u][1].append(lambda u=u: c_tile(u // 2, 0, o_dst))
            else:
                fills[u][1].append(lambda u=u: c_tile(u // 2, 2, o_dst))
                fills[u][2].append(lambda u=u: c_tile(u // 2, 1, o_dst))

    def hosts_tile(u, k):
        return k == 1 or (k == 2 and u % 2 == 1)

    def run_plain(parts, todo, small=()):
        per = -(-len(todo) // (len(parts) - 1))
        nh, ns, b = len(parts) - 3, len(small), 0
        for n, part in enumerate(parts):
            while b < ns and b * nh <= n * ns:
                small[b]()
                b += 1
            part()
            meter(todo, per)
        assert b == ns and not todo

    def run_cb(slot, q_src, o_dst, parts, todo, nlead, ntrail, mid):
        ev = (0, 8, 4, 12, 2, 10, 6, 14)
        cand = [(u, 1) for u in range(NU)] + [(NU, 0)] * ntrail + [(u, 2) for u in range(1, NU, 2)]
        cand += [(u, 2) for u in ev] + [(u + 1, 3) for u in ev] + [(u, 3) for u in ev]
        pos = sorted(cand[:len(parts) - nlead])
        quiet = [p for p in pos if p[0] < NU and not hosts_tile(*p)]
        edge = -(-(len(todo) - mid * len(quiet)) // (nlead + ntrail))
        for part in parts[:nlead]:
            part()
            meter(todo, edge)
        fills = empty_fills()
        for part, (u, k) in zip(parts[nlead:], pos):
            fills[u][k].append(part)
            if (u, k) in quiet:
                fills[u][k].append(lambda: meter(todo, mid))
            elif u == NU:
                fills[u][k].append(lambda: meter(todo, edge))
        tile_fills(fills, o_dst)
        run_slots(cb_ops(slot, q_src), fills)
        assert not todo

    cp_wq(0, 0, 0).start()
    cp_xa(0).start()
    cp_xa(1).start()
    cp_wq(0, 1, 1).start()
    cp_wq(0, 2, 2).start()
    cp_xa(2).start()
    cp_xa(3).start()
    cp_k(0, 0, 0).start()
    cp_wq(0, 3, 3).start()
    cp_v(0, 0, 1).start()
    cp_k(0, 1, 1).start()
    cp_wo(0, 0, 1).start()
    cp_v(0, 1, 2).start()
    cp_k(0, 2, 2).start()
    cp_wo(0, 1, 2).start()
    gmax[...] = jnp.zeros(gmax.shape, f32)

    def zinit(i, carry):
        zero[i % 2] = jnp.zeros((8, DH), u32)
        flag[i % 3] = 0
        acc[1, i // 2, i % 2] = jnp.zeros((MQ, KH), f32)
        return carry
    lax.fori_loop(0, 14, zinit, 0)

    def block(fn):
        pl.when(flag[0] == 0)(fn)

    def a_str(lo, hi, slab, dst):
        return [piece(n, [(xs.at[0], ws.at[slab])], dst, False) for n in range(lo, hi)]

    cp_wq(0, 0, 0).wait()

    def quarter(i, carry):
        @pl.when(i == 2)
        def _():
            cp_wq(0, 0, 1).wait()
            cp_wq(0, 0, 2).wait()
            run_plain([p for u in range(4) for p in a_plain(u, 1, q_alt, x_buf.at[0])],
                      w_todo(wq_buf.at[1], ws.at[4]) + w_todo(wq_buf.at[2], ws.at[5]))
            cp_wq(0, 4, 2).start()
        cp_xa(i).wait()
        xq = x_buf.at[0, pl.ds(pl.multiple_of(i * 2 * CR, 2 * CR), 2 * CR)]
        qq = q_scr.at[pl.ds(pl.multiple_of(i * CR, CR), CR)]
        run_plain([p for u in range(4) for p in a_plain(u, 0, qq, xq)], x_todo(2 * i))
        return carry
    lax.fori_loop(0, 4, quarter, 0)

    cp_k(0, 0, 0).wait()
    cp_wq(0, 0, 3).wait()

    @block
    def _():
        run_plain(a_str(7, ND, 4, qm1) + a_str(0, 11, 5, qm2), w_todo(wq_buf.at[3], ws.at[6]),
                  [(lambda b=b: stage_b(b, 0, lambda b: q_scr)) for b in range(B)])

    cp_v(0, 0, 1).wait()
    cp_k(0, 0, 1).wait()
    cp_wo(0, 0, 1).wait()

    @block
    def _():
        issue_packet_static(3)
        issue_packet_static(4)
        cp_xb().start()
        run_cb(1, lambda b: q_alt if b < 8 else qm1, o_alt,
               a_str(11, ND, 5, qm2) + a_str(0, 17, 6, qm), w_todo(wo_buf.at[1], ws.at[7]), 0, 3, 5)

    wait_packet(2)

    @block
    def _():
        d0 = [piece(n, [(o_alt, ws.at[7])], acc.at[0], False) for n in range(ND)]
        run_cb(2, lambda b: qm2, o_scr, d0 + a_str(17, ND, 6, qm),
               w_todo(wo_buf.at[2], ws.at[0]) + w_todo(wq_buf.at[2], ws.at[2]), 3, 4, 7)

    def body(t, carry):
        slot = t & (NBUF - 1)

        @pl.when(t == T_XB)
        def _():
            cp_xb().wait()

            def xb(c, carry2):
                for tile in range(3):
                    x_ops(1, c, tile)
                return carry2
            lax.fori_loop(0, NC, xb, 0)

        wait_packet(slot)
        xbr = (t + 1) >> 3
        abr = (t - 2) >> 3
        win = ws.at[pl.ds(t - T0, 4)]
        todo = w_todo(wo_buf.at[slot], win.at[1]) + w_todo(wq_buf.at[slot], win.at[3])
        dp = [piece(n, [(o_scr, win.at[0])], acc.at[abr], True) for n in range(ND)]
        ap = [piece(n, [(xs.at[xbr], win.at[2])], qm, False) for n in range(ND)]
        plan = [(f, (0, 0)) for f in dp[:3]] + [(f, (0, 1)) for f in dp[3:7]]
        quarters = [dp[7:17],
                    [x for pair in zip(ap[:4], dp[17:21]) for x in pair] + ap[4:7],
                    [x for pair in zip(dp[21:25], ap[7:11]) for x in pair] + dp[25:28],
                    ap[11:21]]
        p10 = [(0, 1), (0, 2), (1, 1), (1, 2), (1, 3), (2, 1), (2, 2), (3, 1), (3, 2), (3, 3)]
        p11 = [(0, 1), (0, 2), (0, 3), (1, 1), (1, 2), (1, 3), (2, 1), (2, 2), (3, 1), (3, 2), (3, 3)]
        for qi, fs in enumerate(quarters):
            pp = p10 if len(fs) == 10 else p11
            if qi == 0:
                pp = [(0, 2), (0, 3)] + pp[2:]
            plan += [(f, (4 * qi + u, k)) for f, (u, k) in zip(fs, pp)]
        plan += [(f, (NU, 0)) for f in ap[21:]]
        fills = empty_fills()
        for n, (f, (u, k)) in enumerate(plan):
            fills[u][k].append(f)
            if n < 6:
                fills[u][k].append(lambda: meter(todo, 8))
            elif n >= len(plan) - 6:
                fills[u][k].append(lambda n=n: meter(todo, -(-len(todo) // (len(plan) - n))))
            elif u < NU and not hosts_tile(u, k):
                fills[u][k].append(lambda: meter(todo, 1))
        tile_fills(fills, o_scr)
        fills[1][3].append(lambda: issue_packet_dyn(t + 2))
        run_slots(cb_ops(slot, lambda b: qm), fills)
        assert not todo
        return carry

    lax.fori_loop(T0, NT - 1, body, 0)

    slot, slot2 = (NT - 1) % NBUF, NT % NBUF
    base = NT - 1 - T0
    w13, w14, w15 = (o_scr, ws.at[base]), (o_alt, ws.at[base + 2]), (o_scr, ws.at[base + 1])

    def d_piece(n, pairs, after=None):
        return piece(n, pairs, acc.at[1], True, after=after)

    def out_a(n):
        return lambda: combine(0, n // 2, n % 2, pin=True)

    def mid(u0):
        return [(u0, 2), (u0 + 1, 1), (u0 + 1, 2), (u0 + 2, 1), (u0 + 3, 1), (u0 + 3, 2), (u0 + 4, 1)]
    drain_pos = ([(0, 1), (1, 1), (1, 2), (2, 1), (3, 1), (3, 2), (4, 1)] + mid(4) + mid(8)
                 + [(13, 1), (13, 2), (14, 1), (15, 1), (15, 2)] + [(NU, 0)] * 9)

    cp_k(0, 0, slot).wait()
    cp_v(0, 0, slot).wait()
    cp_wo(0, 0, slot2).wait()

    @block
    def _():
        todo = w_todo(wo_buf.at[slot2], ws.at[base + 1])
        seq = [d_piece(21 + k, [w13]) for k in range(7)] + [d_piece(n, [w13, w14]) for n in range(21)]
        fills = empty_fills()
        for n, (f, (u, k)) in enumerate(zip(seq, drain_pos)):
            fills[u][k].append(f)
            if n >= 7:
                fills[u][k].append(out_a(n // 3 - 3) if n % 3 == 0 else (lambda: meter(todo, 4)))
        tile_fills(fills, o_alt)
        run_slots(cb_ops(slot, lambda b: qm), fills)
        assert not todo

    cp_v(0, 0, slot2).wait()

    @block
    def _():
        ok = jnp.max(gmax[...]) * SCALE <= LOGIT_LIMIT
        flag[2] = jnp.where(ok, 0, 1)

        def fin(sc, k):
            return {4: (lambda: combine(1, sc, 0)), 6: (lambda: combine(1, sc, 1))}.get(k)
        seq = [d_piece(21 + k, [w14]) for k in range(7)]
        seq += [d_piece(n, [w15], fin(*divmod(n, 7))) for n in range(ND)]
        fills = empty_fills()
        for n, (f, (u, k)) in enumerate(zip(seq, drain_pos)):
            fills[u][k].append(f)
            if n == 0:
                fills[u][k].append(out_a(2 * NSC - 1))
        tile_fills(fills, o_scr)
        run_slots(cb_ops(slot2, None), fills)

    for br in range(2):
        for sc in range(NSC):
            for half in range(2):
                for pr in (range(4) if is_last(br, sc, half) else [None]):
                    cp_out(br, sc, half, pr).wait()

    @pl.when(flag[2] != 0)
    def _():
        def fstep(t, carry):
            br, hg = t // NS, t % NS
            for j in range(2):
                @pl.when(br == j)
                def _():
                    for cp in (cp_wq, cp_k, cp_v, cp_wo):
                        cp(j, hg, 0).start()
            wait_packet(0)

            def fbatch(b, carry2):
                rows = pl.ds(pl.multiple_of(b * SQ, SQ), SQ)
                q = _dot(x_buf[br, rows, :], wq_buf[0])
                oh = []
                for h in range(HG):
                    p, _ = _softmax(q[:, h * DH:(h + 1) * DH].astype(bf16), k_buf[0, b, h])
                    oh.append(_dot(p[:, :SK].astype(bf16), v_buf[0, b, h]))
                upd = _dot(jnp.concatenate(oh, axis=1).astype(bf16), wo_buf[0])
                ar = pl.ds(pl.multiple_of((b % 8) * SQ, SQ), SQ)
                for half in range(2):
                    prev = jnp.where(hg == 0, 0.0, acc[br, b // 8, half, ar, :])
                    new = prev + upd[:, half * KH:(half + 1) * KH]
                    acc[br, b // 8, half, ar, :] = new
                    ostage[br, rows, half * KH:(half + 1) * KH] = new.astype(bf16)
                return carry2
            lax.fori_loop(0, B, fbatch, 0)
            return carry
        lax.fori_loop(0, NT, fstep, 0)
        outs = [cp_out(br, sc, half) for br in range(2) for sc in range(NSC) for half in range(2)]
        for cp in outs:
            cp.start()
        for cp in outs:
            cp.wait()


@jax.jit
def pallas_concat_heads__gqa_block_cached__gqa_block_cached__near_ridge_kernel(
    A_x: jax.Array,
    A_k_cache: jax.Array,
    A_v_cache: jax.Array,
    A_wq: jax.Array,
    A_wo: jax.Array,
    B_x: jax.Array,
    B_k_cache: jax.Array,
    B_v_cache: jax.Array,
    B_wq: jax.Array,
    B_wo: jax.Array,
):
    out = pl.pallas_call(
        _kernel,
        in_specs=[pl.BlockSpec(memory_space=pl.ANY)] * 10,
        out_specs=pl.BlockSpec(memory_space=pl.ANY),
        out_shape=jax.ShapeDtypeStruct((M, 2 * D), bf16),
        scratch_shapes=[
            pltpu.VMEM((2, M, D), bf16),
            pltpu.VMEM((NBUF, B, HG, SK, DH), bf16),
            pltpu.VMEM((NBUF, B, HG, SK, DH), bf16),
            pltpu.VMEM((NBUF, D, W), bf16),
            pltpu.VMEM((NBUF, W, D), bf16),
            pltpu.VMEM((M // 2, W), u32),
            pltpu.VMEM((M // 2, W), u32),
            pltpu.VMEM((M // 2, W), u32),
            pltpu.VMEM((MQ // 2, 49 * DH), u32),
            pltpu.VMEM((MQ // 2, 49 * DH), u32),
            pltpu.VMEM((2, MQ // 2, 49 * DH), u32),
            pltpu.VMEM((NT - 1, DH // 2, 49 * DH), u32),
            pltpu.VMEM((7, 2, MQ, KH), f32),
            pltpu.VMEM((7, 2, MQ, KH), f32),
            pltpu.VMEM((7, 2, MQ, KH), f32),
            pltpu.VMEM((2, 7, 2, MQ, KH), f32),
            pltpu.VMEM((2, M, D), bf16),
            pltpu.VMEM((B, 8, DH), f32),
            pltpu.VMEM((2, 8, DH), u32),
            pltpu.SMEM((3,), jnp.int32),
            pltpu.SemaphoreType.DMA((NSEM,)),
        ],
        compiler_params=pltpu.CompilerParams(
            vmem_limit_bytes=110 * 1024 * 1024,
            disable_bounds_checks=True, disable_semaphore_checks=True),
    )(A_x.reshape(M, D), A_k_cache, A_v_cache, A_wq, A_wo,
      B_x.reshape(M, D), B_k_cache, B_v_cache, B_wq, B_wo)
    return out.reshape(B, SQ, 2 * D)
```

```python
import jax
import jax.numpy as jnp
from jax import lax
import jax.experimental.pallas as pl
import jax.experimental.pallas.tpu as pltpu

B, SQ, D = 32, 48, 512
H, SK, DH = 32, 48, 128
HG = 4
R = 4
NS = H // HG
NT = 2 * NS
NC = B // R
NU = 2 * NC
NSC = NC // 2
ND = 7 * NSC
CR = R * SQ
HR = CR // 2
SH = SQ // 2
M = B * SQ
MQ = M // 4
SR = MQ // NSC
W = HG * DH
KH = 256
RB = 16
NBUF = 4
T0 = 3
T_XB = 5
LOGIT_LIMIT = 5.0
SCALE = DH ** -0.5
EXP2_SCALE = SCALE * 1.4426950408889634
f32 = jnp.float32
bf16 = jnp.bfloat16
u32 = jnp.uint32

S_X = 4 * NBUF
S_XB = S_X + 4
S_O = S_XB + 1
NSEM = S_O + 4 * NSC + 3

LHS_TERMS = (((0, 0), (1, 1), 1), ((1, 0), (1, 1), 1), ((0, 0), None, 0), ((1, 1), None, 0),
             ((0, 0), (0, 1), 1), ((1, 0), (0, 0), -1), ((0, 1), (1, 1), -1))
RHS_TERMS = (((0, 0), (1, 1), 1), ((0, 0), None, 0), ((0, 1), (1, 1), -1), ((1, 0), (0, 0), -1),
             ((1, 1), None, 0), ((0, 0), (0, 1), 1), ((1, 0), (1, 1), 1))
IORD = (1, 3, 4, 6, 0, 2, 5)
GROUPS = ((0, 0), (0, 1), (0, 2), (1, 0), (1, 1), (1, 2))


def _pack(v):
    return pltpu.bitcast(v.astype(bf16), u32)


def _unpack(v):
    return pltpu.bitcast(v, bf16)


def _dot(a, b):
    return jnp.dot(a, b, preferred_element_type=f32)


def _lhs_ops(a11, a12, a21, a22):
    return (a11 + a22, a21 + a22, a11, a22, a11 + a12, a21 - a11, a12 - a22)


def _rhs_ops(b11, b12, b21, b22):
    return (b11 + b22, b11, b12 - b22, b21 - b11, b22, b11 + b12, b21 + b22)


def _outer_combine(mm, half, z=None):
    shared = mm(3 if half == 0 else 2)
    if z is not None:
        shared = shared + z
    if half == 0:
        top, bot = (mm(0) + shared) + (mm(6) - mm(4)), mm(1) + shared
    else:
        top, bot = shared + mm(4), (mm(0) - mm(1)) + (shared + mm(5))
    return jnp.concatenate([top, bot], axis=0)


def _softmax(qq, kk):
    s = lax.dot_general(qq, kk, (((1,), (1,)), ((), ())), preferred_element_type=f32)
    s = jnp.concatenate([s, jnp.full((SQ, DH - SK), -jnp.inf, f32)], axis=1)
    m = jnp.max(s, axis=-1, keepdims=True)
    p = jnp.exp2((s - m) * EXP2_SCALE)
    l = jnp.sum(p, axis=-1, keepdims=True)
    r = pl.reciprocal(l, approx=True)
    r = r * (2.0 - l * r)
    return p * r, m


def _aligned(v, n):
    return v if isinstance(v, int) else pl.multiple_of(v, n)


def _kernel(ax, ak, av, awq, awo, bx, bk, bv, bwq, bwo, out_hbm,
            x_buf, k_buf, v_buf, wq_buf, wo_buf, q_scr, q_alt, p_scr, o_scr, o_alt, xs, ws,
            qm, qm1, qm2, acc, ostage, gmax, zero, flag, sem):
    srcs = ((ax, ak, av, awq, awo), (bx, bk, bv, bwq, bwo))

    def cp_wq(br, hg, slot):
        return pltpu.make_async_copy(srcs[br][3].at[:, pl.ds(_aligned(hg * W, W), W)],
                                     wq_buf.at[slot], sem.at[4 * slot])

    def cp_k(br, hg, slot):
        return pltpu.make_async_copy(srcs[br][1].at[:, pl.ds(hg * HG, HG)],
                                     k_buf.at[slot], sem.at[4 * slot + 1])

    def cp_v(br, hg, slot):
        return pltpu.make_async_copy(srcs[br][2].at[:, pl.ds(hg * HG, HG)],
                                     v_buf.at[slot], sem.at[4 * slot + 2])

    def cp_wo(br, hg, slot):
        return pltpu.make_async_copy(srcs[br][4].at[pl.ds(_aligned(hg * W, W), W), :],
                                     wo_buf.at[slot], sem.at[4 * slot + 3])

    def cp_xa(i):
        sl = pl.ds(_aligned(i * 2 * CR, 2 * CR), 2 * CR)
        return pltpu.make_async_copy(ax.at[sl], x_buf.at[0, sl], sem.at[S_X + i])

    def cp_xb():
        return pltpu.make_async_copy(bx, x_buf.at[1], sem.at[S_XB])

    def cp_out(br, sc, half, pr=None):
        if pr is None:
            rows, si = pl.ds(sc * 2 * CR, 2 * CR), (br * NSC + sc) * 2 + half
        else:
            rows, si = pl.ds(sc * 2 * CR + pr * 2 * SQ, 2 * SQ), 4 * NSC - 1 + pr
        return pltpu.make_async_copy(ostage.at[br, rows, pl.ds(half * KH, KH)],
                                     out_hbm.at[rows, pl.ds(br * D + half * KH, KH)],
                                     sem.at[S_O + si])

    def is_last(br, sc, half):
        return (br, sc, half) == (1, NSC - 1, 1)

    def issue_packet_static(p):
        slot = p % NBUF
        cp_wq(0, p + 2, slot).start()
        cp_k(0, p, slot).start()
        cp_v(0, p - 1, slot).start()
        cp_wo(0, p - 1, slot).start()

    def wait_packet(slot):
        cp_wq(0, 0, slot).wait()
        cp_k(0, 0, slot).wait()
        cp_v(0, 0, slot).wait()
        cp_wo(0, 0, slot).wait()

    def issue_packet_dyn(p):
        slot = p & (NBUF - 1)

        @pl.when(p + 2 < NS)
        def _():
            cp_wq(0, p + 2, slot).start()

        @pl.when(jnp.logical_and(p + 2 >= NS, p + 2 < NT))
        def _():
            cp_wq(1, p + 2 - NS, slot).start()

        @pl.when(p + 2 == NT)
        def _():
            pltpu.make_async_copy(bwo.at[pl.ds((NS - 2) * W, W), :], wq_buf.at[slot],
                                  sem.at[4 * slot]).start()

        @pl.when(p < NS)
        def _():
            cp_k(0, p, slot).start()

        @pl.when(jnp.logical_and(p >= NS, p < NT))
        def _():
            cp_k(1, p - NS, slot).start()

        @pl.when(p - 1 < NS)
        def _():
            cp_v(0, p - 1, slot).start()
            cp_wo(0, p - 1, slot).start()

        @pl.when(p - 1 >= NS)
        def _():
            cp_v(1, p - 1 - NS, slot).start()

        @pl.when(jnp.logical_and(p - 1 >= NS, p != NT - 1))
        def _():
            cp_wo(1, p - 1 - NS, slot).start()

    last = {}

    def anchor(v, rows, cols, k=0):
        z = pltpu.bitcast(pltpu.bitcast(v[8 * k:8 * k + 8, :DH], u32) & zero[0], f32)
        if cols > DH:
            z = jnp.concatenate([z] * (cols // DH), axis=1)
        return jnp.concatenate([z] * (rows // 8), axis=0)

    def meter(todo, count):
        src = last['f']
        n = src.shape[0] // 8
        for k in range(count):
            if todo:
                todo.pop(0)(anchor(src, RB, KH, ((k + 1) * n) // count - 1))

    def w_sums(w, dst, j, i, z):
        r = j * RB

        def quad(k1, n1):
            return [w[(2 * k1 + k2) * DH + r:(2 * k1 + k2) * DH + r + RB,
                      n1 * KH:(n1 + 1) * KH].astype(f32) for k2 in range(2)]
        ta, tb, sg = RHS_TERMS[i]
        v = [x + z for x in quad(*ta)]
        if tb is not None:
            v = [x + y if sg > 0 else x - y for x, y in zip(v, quad(*tb))]
        ops = _rhs_ops(v[0][:, :DH], v[0][:, DH:], v[1][:, :DH], v[1][:, DH:])
        dst[r // 2:(r + RB) // 2, i * 7 * DH:(i + 1) * 7 * DH] = _pack(jnp.concatenate(ops, axis=1))

    def w_todo(w, dst):
        return [(lambda z, j=j, i=i: w_sums(w, dst, j, i, z))
                for j in range(DH // RB) for i in range(7)]

    def lhs_group(blk, i, z, dst, r0, nrows):
        ta, tb, sg = LHS_TERMS[i]
        v = {}
        for m2 in range(2):
            for k2 in range(2):
                x = blk(*ta, m2, k2)
                if z is not None and m2 == k2:
                    x = x + z
                if tb is not None:
                    y = blk(*tb, m2, k2)
                    x = x + y if sg > 0 else x - y
                v[m2, k2] = x
        ops = _lhs_ops(v[0, 0], v[0, 1], v[1, 0], v[1, 1])
        dst[r0 // 2:(r0 + nrows) // 2, i * 7 * DH:(i + 1) * 7 * DH] = _pack(jnp.concatenate(ops, axis=1))

    def x_ops(br, c, tile, z=None, outer=range(7)):
        grp = GROUPS[2 * tile:2 * tile + 2]
        xc = x_buf.at[br, pl.ds(_aligned(c * CR, CR), CR)]
        xd = xs.at[br, pl.ds(_aligned(c * SH, SH), SH)]

        def blk(m1, k1, m2, k2):
            out = []
            for q, g in grp:
                r = (2 * q + m2) * SQ + m1 * SH + 8 * g
                out.append(xc[r:r + 8, k1 * KH:(k1 + 1) * KH].astype(f32)[:, k2 * DH:(k2 + 1) * DH])
            return jnp.concatenate(out, axis=0)
        for i in outer:
            lhs_group(blk, i, None if z is None else z[:, :DH], xd, 16 * tile, 16)

    def x_todo(c0):
        return [(lambda z, c=c, tile=tile, i=i: x_ops(0, c0 + c, tile, z, (i,)))
                for c in range(2) for tile in range(3) for i in range(7)]

    def a_plain(u, slot, q_dst, x_src):
        c, nt = divmod(u, 2)
        st = {}

        def p1():
            st['q'] = _dot(x_src[c * CR:(c + 1) * CR, :], wq_buf[slot, :, 2 * nt * DH:(2 * nt + 1) * DH])
            last['f'] = st['q']

        def p2():
            q1 = _dot(x_src[c * CR:(c + 1) * CR, :], wq_buf[slot, :, (2 * nt + 1) * DH:(2 * nt + 2) * DH])
            last['f'] = q1
            q_dst[c * HR:(c + 1) * HR, nt * KH:(nt + 1) * KH] = _pack(jnp.concatenate([st['q'], q1], axis=1))
        return p1, p2

    def stage_b(b, slot, q_src):
        q_src = q_src(b)
        if len(q_src.shape) == 4:
            hs = slice((b // 2) * SH, (b // 2 + 1) * SH)
            vals = [q_src[i, b % 2, hs, :] for i in range(7)]
            qh = [_outer_combine(lambda i: vals[i], half) for half in range(2)]
            qs = [qh[h // 2][:, (h % 2) * DH:(h % 2 + 1) * DH].astype(bf16) for h in range(HG)]
        else:
            qs = [_unpack(q_src[b * SH:(b + 1) * SH, h * DH:(h + 1) * DH]) for h in range(HG)]
        ps, g = [], None
        for h in range(HG):
            p, m = _softmax(qs[h], k_buf[slot, b, h])
            ps.append(p)
            am = jnp.abs(m)
            am = jnp.maximum(am[:SH], am[SH:])
            g = am if g is None else jnp.maximum(g, am)
        g = jnp.maximum(jnp.maximum(g[:8], g[8:16]), g[16:])
        p_scr[b * SH:(b + 1) * SH, :] = _pack(jnp.concatenate(ps, axis=1))
        gmax[b] = jnp.maximum(gmax[b], jnp.broadcast_to(g, (8, DH)))

    o_val = {}

    def stage_c(b, slot):
        for h in range(HG):
            p = _unpack(p_scr[b * SH:(b + 1) * SH, h * DH:(h + 1) * DH])[:, :SK]
            o_val[b, h] = _dot(p, v_buf[slot, b, h])

    def c_tile(c, tile, o_dst):
        anc = last['f']
        grp = GROUPS[2 * tile:2 * tile + 2]
        n = anc.shape[0] // 8

        blocks = {}

        def blk(*key):
            m1, k1, m2, k2 = key
            if key not in blocks:
                v = [o_val[c * R + 2 * q + m2, 2 * k1 + k2] for q, _ in grp]
                r = [m1 * SH + 8 * g for _, g in grp]
                if tile == 1:
                    blocks[key] = jnp.concatenate([v[0][r[0]:r[0] + 8], v[1][r[1]:r[1] + 8]], axis=0)
                else:
                    blocks[key] = v[0][r[0]:r[0] + 16]
            return blocks[key]
        for i in range(7):
            lhs_group(blk, i, anchor(anc, 16, DH, (i * n) // 7), o_dst, c * SQ + 16 * tile, 16)

    def piece(n, pairs, dst, accumulate, after=None):
        sc, i = n // 7, IORD[n % 7]
        rows = slice(sc * SR // 2, (sc + 1) * SR // 2)
        hs = slice(sc * SR, (sc + 1) * SR)

        def mm(k):
            cols = slice((i * 7 + k) * DH, (i * 7 + k + 1) * DH)
            return _dot(_unpack(jnp.concatenate([o[rows, cols] for o, _ in pairs], axis=1)),
                        _unpack(jnp.concatenate([w[:, cols] for _, w in pairs], axis=0)))

        def run():
            m2, m4, m3, m5 = mm(1), mm(3), mm(2), mm(4)
            t11, t22, s34 = m4 - m5, m3 - m2, m3 + m4
            c21, c12 = s34 - t22, s34 - t11
            m1, m7, m6 = mm(0), mm(6), mm(5)
            last['f'] = jnp.concatenate([m2, m1], axis=0)
            top = jnp.concatenate([t11 + (m1 + m7), c12], axis=1)
            bot = jnp.concatenate([c21, t22 + (m1 + m6)], axis=1)
            if accumulate:
                top, bot = dst[i, 0, hs, :] + top, dst[i, 1, hs, :] + bot
            dst[i, 0, hs, :] = top
            dst[i, 1, hs, :] = bot
            if after is not None:
                after()
        return run

    def combine(br, sc, half, pin=False):
        anc = last['f']
        for pr in range(4):
            hs = slice(sc * SR + pr * SH, sc * SR + (pr + 1) * SH)
            for m2 in range(2):
                z = anchor(anc, SH, KH, 3 * (2 * pr + m2)) if pin else None
                v = _outer_combine(lambda i: acc[br, i, m2, hs, :], half, z)
                b = sc * 8 + 2 * pr + m2
                ostage[br, b * SQ:(b + 1) * SQ, half * KH:(half + 1) * KH] = v.astype(bf16)
            if is_last(br, sc, half):
                cp_out(br, sc, half, pr).start()
        if not is_last(br, sc, half):
            cp_out(br, sc, half).start()

    def run_slots(ops, fills):
        for u in range(len(fills)):
            for op, fl in zip(ops(u), fills[u]):
                if op is not None:
                    op()
                for f in fl:
                    f()

    def empty_fills():
        return [[[], [], [], []] for _ in range(NU + 1)]

    def cb_ops(slot, q_src):
        def ops(u):
            if u >= NU:
                return [None] * 4
            out = [lambda: stage_c(2 * u, slot), lambda: stage_c(2 * u + 1, slot)]
            if q_src is None:
                return out + [None, None]
            return out + [lambda: stage_b(2 * u, slot, q_src), lambda: stage_b(2 * u + 1, slot, q_src)]
        return ops

    def tile_fills(fills, o_dst):
        for u in range(NU):
            if u % 2 == 0:
                fills[u][1].append(lambda u=u: c_tile(u // 2, 0, o_dst))
            else:
                fills[u][1].append(lambda u=u: c_tile(u // 2, 2, o_dst))
                fills[u][2].append(lambda u=u: c_tile(u // 2, 1, o_dst))

    def hosts_tile(u, k):
        return k == 1 or (k == 2 and u % 2 == 1)

    def run_plain(parts, todo, small=()):
        per = -(-len(todo) // (len(parts) - 1))
        nh, ns, b = len(parts) - 3, len(small), 0
        for n, part in enumerate(parts):
            while b < ns and b * nh <= n * ns:
                small[b]()
                b += 1
            part()
            meter(todo, per)
        assert b == ns and not todo

    def run_cb(slot, q_src, o_dst, parts, todo, nlead, ntrail, mid):
        ev = (0, 8, 4, 12, 2, 10, 6, 14)
        cand = [(u, 1) for u in range(NU)] + [(NU, 0)] * ntrail + [(u, 2) for u in range(1, NU, 2)]
        cand += [(u, 2) for u in ev] + [(u + 1, 3) for u in ev] + [(u, 3) for u in ev]
        pos = sorted(cand[:len(parts) - nlead])
        quiet = [p for p in pos if p[0] < NU and not hosts_tile(*p)]
        edge = -(-(len(todo) - mid * len(quiet)) // (nlead + ntrail))
        for part in parts[:nlead]:
            part()
            meter(todo, edge)
        fills = empty_fills()
        for part, (u, k) in zip(parts[nlead:], pos):
            fills[u][k].append(part)
            if (u, k) in quiet:
                fills[u][k].append(lambda: meter(todo, mid))
            elif u == NU:
                fills[u][k].append(lambda: meter(todo, edge))
        tile_fills(fills, o_dst)
        run_slots(cb_ops(slot, q_src), fills)
        assert not todo

    cp_wq(0, 0, 0).start()
    cp_xa(0).start()
    cp_xa(1).start()
    cp_wq(0, 1, 1).start()
    cp_wq(0, 2, 2).start()
    cp_xa(2).start()
    cp_xa(3).start()
    cp_k(0, 0, 0).start()
    cp_wq(0, 3, 3).start()
    cp_v(0, 0, 1).start()
    cp_k(0, 1, 1).start()
    cp_wo(0, 0, 1).start()
    cp_v(0, 1, 2).start()
    cp_k(0, 2, 2).start()
    cp_wo(0, 1, 2).start()
    gmax[...] = jnp.zeros(gmax.shape, f32)

    def zinit(i, carry):
        zero[i % 2] = jnp.zeros((8, DH), u32)
        flag[i % 3] = 0
        acc[1, i // 2, i % 2] = jnp.zeros((MQ, KH), f32)
        return carry
    lax.fori_loop(0, 14, zinit, 0)

    def block(fn):
        pl.when(flag[0] == 0)(fn)

    def a_str(lo, hi, slab, dst):
        return [piece(n, [(xs.at[0], ws.at[slab])], dst, False) for n in range(lo, hi)]

    cp_wq(0, 0, 0).wait()

    def quarter(i, carry):
        @pl.when(i == 2)
        def _():
            cp_wq(0, 0, 1).wait()
            cp_wq(0, 0, 2).wait()
            run_plain([p for u in range(4) for p in a_plain(u, 1, q_alt, x_buf.at[0])],
                      w_todo(wq_buf.at[1], ws.at[4]) + w_todo(wq_buf.at[2], ws.at[5]))
            cp_wq(0, 4, 2).start()
        cp_xa(i).wait()
        xq = x_buf.at[0, pl.ds(pl.multiple_of(i * 2 * CR, 2 * CR), 2 * CR)]
        qq = q_scr.at[pl.ds(pl.multiple_of(i * CR, CR), CR)]
        run_plain([p for u in range(4) for p in a_plain(u, 0, qq, xq)], x_todo(2 * i))
        return carry
    lax.fori_loop(0, 4, quarter, 0)

    cp_k(0, 0, 0).wait()
    cp_wq(0, 0, 3).wait()

    @block
    def _():
        run_plain(a_str(7, ND, 4, qm1) + a_str(0, 11, 5, qm2), w_todo(wq_buf.at[3], ws.at[6]),
                  [(lambda b=b: stage_b(b, 0, lambda b: q_scr)) for b in range(B)])

    cp_v(0, 0, 1).wait()
    cp_k(0, 0, 1).wait()
    cp_wo(0, 0, 1).wait()

    @block
    def _():
        issue_packet_static(3)
        issue_packet_static(4)
        cp_xb().start()
        run_cb(1, lambda b: q_alt if b < 8 else qm1, o_alt,
               a_str(11, ND, 5, qm2) + a_str(0, 17, 6, qm), w_todo(wo_buf.at[1], ws.at[7]), 0, 3, 5)

    wait_packet(2)

    @block
    def _():
        d0 = [piece(n, [(o_alt, ws.at[7])], acc.at[0], False) for n in range(ND)]
        run_cb(2, lambda b: qm2, o_scr, d0 + a_str(17, ND, 6, qm),
               w_todo(wo_buf.at[2], ws.at[0]) + w_todo(wq_buf.at[2], ws.at[2]), 3, 4, 7)

    def body(t, carry):
        slot = t & (NBUF - 1)

        @pl.when(t == T_XB)
        def _():
            cp_xb().wait()

            def xb(c, carry2):
                for tile in range(3):
                    x_ops(1, c, tile)
                return carry2
            lax.fori_loop(0, NC, xb, 0)

        wait_packet(slot)
        xbr = (t + 1) >> 3
        abr = (t - 2) >> 3
        win = ws.at[pl.ds(t - T0, 4)]
        todo = w_todo(wo_buf.at[slot], win.at[1]) + w_todo(wq_buf.at[slot], win.at[3])
        dp = [piece(n, [(o_scr, win.at[0])], acc.at[abr], True) for n in range(ND)]
        ap = [piece(n, [(xs.at[xbr], win.at[2])], qm, False) for n in range(ND)]
        plan = [(f, (0, 0)) for f in dp[:3]] + [(f, (0, 1)) for f in dp[3:7]]
        quarters = [dp[7:17],
                    [x for pair in zip(ap[:4], dp[17:21]) for x in pair] + ap[4:7],
                    [x for pair in zip(dp[21:25], ap[7:11]) for x in pair] + dp[25:28],
                    ap[11:21]]
        p10 = [(0, 1), (0, 2), (1, 1), (1, 2), (1, 3), (2, 1), (2, 2), (3, 1), (3, 2), (3, 3)]
        p11 = [(0, 1), (0, 2), (0, 3), (1, 1), (1, 2), (1, 3), (2, 1), (2, 2), (3, 1), (3, 2), (3, 3)]
        for qi, fs in enumerate(quarters):
            pp = p10 if len(fs) == 10 else p11
            if qi == 0:
                pp = [(0, 2), (0, 3)] + pp[2:]
            plan += [(f, (4 * qi + u, k)) for f, (u, k) in zip(fs, pp)]
        plan += [(f, (NU, 0)) for f in ap[21:]]
        fills = empty_fills()
        for n, (f, (u, k)) in enumerate(plan):
            fills[u][k].append(f)
            if n < 6:
                fills[u][k].append(lambda: meter(todo, 8))
            elif n >= len(plan) - 6:
                fills[u][k].append(lambda n=n: meter(todo, -(-len(todo) // (len(plan) - n))))
            elif u < NU and not hosts_tile(u, k):
                fills[u][k].append(lambda: meter(todo, 1))
        tile_fills(fills, o_scr)
        fills[1][3].append(lambda: issue_packet_dyn(t + 2))
        run_slots(cb_ops(slot, lambda b: qm), fills)
        assert not todo
        return carry

    lax.fori_loop(T0, NT - 1, body, 0)

    slot, slot2 = (NT - 1) % NBUF, NT % NBUF
    base = NT - 1 - T0
    w13, w14, w15 = (o_scr, ws.at[base]), (o_alt, ws.at[base + 2]), (o_scr, ws.at[base + 1])

    def d_piece(n, pairs, after=None):
        return piece(n, pairs, acc.at[1], True, after=after)

    def out_a(n):
        return lambda: combine(0, n // 2, n % 2, pin=True)

    def mid(u0):
        return [(u0, 2), (u0 + 1, 1), (u0 + 1, 2), (u0 + 2, 1), (u0 + 3, 1), (u0 + 3, 2), (u0 + 4, 1)]
    drain_pos = ([(0, 1), (1, 1), (1, 2), (2, 1), (3, 1), (3, 2), (4, 1)] + mid(4) + mid(8)
                 + [(13, 1), (13, 2), (14, 1), (15, 1), (15, 2)] + [(NU, 0)] * 9)

    cp_k(0, 0, slot).wait()
    cp_v(0, 0, slot).wait()
    cp_wo(0, 0, slot2).wait()

    @block
    def _():
        todo = w_todo(wo_buf.at[slot2], ws.at[base + 1])
        seq = [d_piece(21 + k, [w13]) for k in range(7)] + [d_piece(n, [w13, w14]) for n in range(21)]
        fills = empty_fills()
        for n, (f, (u, k)) in enumerate(zip(seq, drain_pos)):
            fills[u][k].append(f)
            if n >= 7:
                fills[u][k].append(out_a(n // 3 - 3) if n % 3 == 0 else (lambda: meter(todo, 4)))
        tile_fills(fills, o_alt)
        run_slots(cb_ops(slot, lambda b: qm), fills)
        assert not todo

    cp_v(0, 0, slot2).wait()

    @block
    def _():
        ok = jnp.max(gmax[...]) * SCALE <= LOGIT_LIMIT
        flag[2] = jnp.where(ok, 0, 1)

        def fin(sc, k):
            return {4: (lambda: combine(1, sc, 0)), 6: (lambda: combine(1, sc, 1))}.get(k)
        seq = [d_piece(21 + k, [w14]) for k in range(7)]
        seq += [d_piece(n, [w15], fin(*divmod(n, 7))) for n in range(ND)]
        fills = empty_fills()
        for n, (f, (u, k)) in enumerate(zip(seq, drain_pos)):
            fills[u][k].append(f)
            if n == 0:
                fills[u][k].append(out_a(2 * NSC - 1))
        tile_fills(fills, o_scr)
        run_slots(cb_ops(slot2, None), fills)

    for br in range(2):
        for sc in range(NSC):
            for half in range(2):
                for pr in (range(4) if is_last(br, sc, half) else [None]):
                    cp_out(br, sc, half, pr).wait()

    @pl.when(flag[2] != 0)
    def _():
        def fstep(t, carry):
            br, hg = t // NS, t % NS
            for j in range(2):
                @pl.when(br == j)
                def _():
                    for cp in (cp_wq, cp_k, cp_v, cp_wo):
                        cp(j, hg, 0).start()
            wait_packet(0)

            def fbatch(b, carry2):
                rows = pl.ds(pl.multiple_of(b * SQ, SQ), SQ)
                q = _dot(x_buf[br, rows, :], wq_buf[0])
                oh = []
                for h in range(HG):
                    p, _ = _softmax(q[:, h * DH:(h + 1) * DH].astype(bf16), k_buf[0, b, h])
                    oh.append(_dot(p[:, :SK].astype(bf16), v_buf[0, b, h]))
                upd = _dot(jnp.concatenate(oh, axis=1).astype(bf16), wo_buf[0])
                ar = pl.ds(pl.multiple_of((b % 8) * SQ, SQ), SQ)
                for half in range(2):
                    prev = jnp.where(hg == 0, 0.0, acc[br, b // 8, half, ar, :])
                    new = prev + upd[:, half * KH:(half + 1) * KH]
                    acc[br, b // 8, half, ar, :] = new
                    ostage[br, rows, half * KH:(half + 1) * KH] = new.astype(bf16)
                return carry2
            lax.fori_loop(0, B, fbatch, 0)
            return carry
        lax.fori_loop(0, NT, fstep, 0)
        outs = [cp_out(br, sc, half) for br in range(2) for sc in range(NSC) for half in range(2)]
        for cp in outs:
            cp.start()
        for cp in outs:
            cp.wait()


@jax.jit
def pallas_concat_heads__gqa_block_cached__gqa_block_cached__near_ridge_kernel(
    A_x: jax.Array,
    A_k_cache: jax.Array,
    A_v_cache: jax.Array,
    A_wq: jax.Array,
    A_wo: jax.Array,
    B_x: jax.Array,
    B_k_cache: jax.Array,
    B_v_cache: jax.Array,
    B_wq: jax.Array,
    B_wo: jax.Array,
):
    out = pl.pallas_call(
        _kernel,
        in_specs=[pl.BlockSpec(memory_space=pl.ANY)] * 10,
        out_specs=pl.BlockSpec(memory_space=pl.ANY),
        out_shape=jax.ShapeDtypeStruct((M, 2 * D), bf16),
        scratch_shapes=[
            pltpu.VMEM((2, M, D), bf16),
            pltpu.VMEM((NBUF, B, HG, SK, DH), bf16),
            pltpu.VMEM((NBUF, B, HG, SK, DH), bf16),
            pltpu.VMEM((NBUF, D, W), bf16),
            pltpu.VMEM((NBUF, W, D), bf16),
            pltpu.VMEM((M // 2, W), u32),
            pltpu.VMEM((M // 2, W), u32),
            pltpu.VMEM((M // 2, W), u32),
            pltpu.VMEM((MQ // 2, 49 * DH), u32),
            pltpu.VMEM((MQ // 2, 49 * DH), u32),
            pltpu.VMEM((2, MQ // 2, 49 * DH), u32),
            pltpu.VMEM((NT - 1, DH // 2, 49 * DH), u32),
            pltpu.VMEM((7, 2, MQ, KH), f32),
            pltpu.VMEM((7, 2, MQ, KH), f32),
            pltpu.VMEM((7, 2, MQ, KH), f32),
            pltpu.VMEM((2, 7, 2, MQ, KH), f32),
            pltpu.VMEM((2, M, D), bf16),
            pltpu.VMEM((B, 8, DH), f32),
            pltpu.VMEM((2, 8, DH), u32),
            pltpu.SMEM((3,), jnp.int32),
            pltpu.SemaphoreType.DMA((NSEM,)),
        ],
        compiler_params=pltpu.CompilerParams(
            vmem_limit_bytes=110 * 1024 * 1024,
            disable_bounds_checks=True, disable_semaphore_checks=True),
    )(A_x.reshape(M, D), A_k_cache, A_v_cache, A_wq, A_wo,
      B_x.reshape(M, D), B_k_cache, B_v_cache, B_wq, B_wo)
    return out.reshape(B, SQ, 2 * D)
```
